```python
import os as _os
_os.environ.setdefault('JAX_PLATFORMS', 'cpu')
import jax
import jax.numpy as jnp

def _softmax(x, axis=-1):
    return jax.nn.softmax(x, axis=axis)

def _gelu(x):
    return jax.nn.gelu(x, approximate=True)

def _silu(x):
    return jax.nn.silu(x)

def _sigmoid(x):
    return jax.nn.sigmoid(x)

def _layernorm(x, axis=-1, eps=1e-05):
    m = jnp.mean(x, axis=axis, keepdims=True)
    v = jnp.var(x, axis=axis, keepdims=True)
    return (x - m) / jnp.sqrt(v + eps)

def _scatter_add(tgt, idx, src, axis=0):
    return tgt.at[idx].add(src)

def _segment_sum(src, seg, n):
    return jax.ops.segment_sum(src, seg, n)

class _Rng:

    def __init__(self, key):
        self._k = key

    def _next(self):
        self._k, sub = jax.random.split(self._k)
        return sub

    def normal(self, shape):
        return jax.random.normal(self._next(), shape, dtype=jnp.bfloat16)

    def randint(self, lo, hi, shape):
        return jax.random.randint(self._next(), shape, lo, hi, dtype=jnp.int32)

    def uniform(self, shape, lo=0.0, hi=1.0):
        return jax.random.uniform(self._next(), shape, jnp.bfloat16, lo, hi)

    def permutation(self, n):
        return jax.random.permutation(self._next(), n)
kernel_name = 'adaLN_cond__mha_block__dense_activation_squared_relu__prompt'

def setup_inputs():
    _rng = _Rng(jax.random.key(int.from_bytes(__import__("os").urandom(4), "little")))
    _w = lambda a: (lambda t: t.astype(jnp.bfloat16) if jnp.issubdtype(t.dtype, jnp.floating) else t)(jnp.asarray(a))

    def _A_setup():
        B, S, D, H = (1, 2048, 512, 32)
        return {'x': _w((lambda *s: _rng.normal(s) * 0.05)(B, S, D)), 'wqkv': _w((lambda *s: _rng.normal(s) * 0.1)(D, 3 * D)), 'wo': _w((lambda *s: _rng.normal(s) * 0.05)(D, D))}
    _A_in = _A_setup()

    def _B_setup():
        B, S, D, F = (1, 2048, 512, 1792)
        return {'x': _w((lambda *s: _rng.normal(s) * 0.05)(B, S, D)), 'w1': _w((lambda *s: _rng.normal(s) * 0.05)(D, F)), 'b1': _w((lambda *s: _rng.normal(s) * 0.05)(F)), 'w2': _w((lambda *s: _rng.normal(s) * 0.05)(F, D)), 'b2': _w((lambda *s: _rng.normal(s) * 0.05)(D))}
    _B_in = _B_setup()
    return {'A_x': _A_in['x'], 'A_wqkv': _A_in['wqkv'], 'A_wo': _A_in['wo'], 'B_x': _B_in['x'], 'B_w1': _B_in['w1'], 'B_b1': _B_in['b1'], 'B_w2': _B_in['w2'], 'B_b2': _B_in['b2'], 'c': _w((lambda *s: _rng.normal(s) * 0.05)(1, 512) * 8.0), 'w_mod': _w((lambda *s: _rng.normal(s) * 0.05)(512, 6 * 512) * 512 ** (-0.5) * 8.0)}

def reference(A_x, A_wqkv, A_wo, B_x, B_w1, B_b1, B_w2, B_b2, c, w_mod):

    def _A_ref(x, wqkv, wo):
        B, S, D = x.shape
        H = 32
        Dh = D // H
        qkv = (lambda x, *d: x.transpose(*d))((x @ wqkv).reshape(B, S, 3, H, Dh), 2, 0, 3, 1, 4)
        q, k, v = (qkv[0], qkv[1], qkv[2])
        scores = jnp.einsum('bhqd,bhkd->bhqk', q, k) * Dh ** (-0.5)
        p = _softmax(scores, axis=-1)
        o = jnp.einsum('bhqk,bhkd->bhqd', p, v)
        return (lambda x, *d: x.transpose(*d))(o, 0, 2, 1, 3).reshape(B, S, D) @ wo

    def _B_ref(x, w1, b1, w2, b2):
        h = jnp.einsum('bsd,df->bsf', x, w1) + b1
        zero = jnp.zeros_like(h)
        r = jnp.where(h > zero, h, zero)
        h = r * r
        out = jnp.einsum('bsf,fd->bsd', h, w2) + b2
        return out
    x = A_x
    mod = (_silu(c) @ w_mod).reshape(c.shape[0], 6, 1, -1)
    sa, ca, ga, sb, cb, gb = (mod[:, 0].copy(), mod[:, 1].copy(), mod[:, 2].copy(), mod[:, 3].copy(), mod[:, 4].copy(), mod[:, 5].copy())
    h = _layernorm(x, axis=-1) * (1 + ca) + sa
    x = x + ga * _A_ref(h, A_wqkv, A_wo)
    h = _layernorm(x, axis=-1) * (1 + cb) + sb
    x = x + gb * _B_ref(h, B_w1, B_b1, B_w2, B_b2)
    return x
```

```python
import functools
import math

import jax
import jax.numpy as jnp
from jax import lax
import jax.experimental.pallas as pl
import jax.experimental.pallas.tpu as pltpu

S = 2048
D = 512
H = 32
DH = 16
F = 1792
HG = 128 // DH
NG = H // HG
EPS = 1e-5
LOG2E = math.log2(math.e)


def _ln(x):
    m = jnp.mean(x, axis=-1, keepdims=True)
    xc = x - m
    v = jnp.mean(xc * xc, axis=-1, keepdims=True)
    return xc * lax.rsqrt(v + EPS)


def _kernel(x_ref, wqkv_ref, wo_ref, w1_ref, b1_ref, w2_ref, b2_ref, c_ref, wmod_ref,
            o_ref, mod_scr, q_scr, k_scr, vt_scr, ot_scr, *, tq, tp):
    i = pl.program_id(0)

    @pl.when(i == 0)
    def _prologue():
        c = c_ref[...].astype(jnp.float32)
        sc = (c * jax.nn.sigmoid(c)).astype(jnp.bfloat16)
        mod = jnp.dot(sc, wmod_ref[...], preferred_element_type=jnp.float32)
        mod_scr[...] = mod.astype(jnp.bfloat16).astype(jnp.float32)
        sa = mod_scr[0:1, 0 * D:1 * D]
        ca = mod_scr[0:1, 1 * D:2 * D]
        row = lax.broadcasted_iota(jnp.int32, (16, S), 0)
        tail = jnp.where(row == 0, 1.0, 0.0).astype(jnp.bfloat16)
        for h in range(H):
            vt_scr[h, 16:32, :] = tail
        for r in range(S // tp):
            rows = pl.ds(r * tp, tp)
            xb = x_ref[rows, :].astype(jnp.float32)
            hb = (_ln(xb) * (1.0 + ca) + sa).astype(jnp.bfloat16)
            qkv = jnp.dot(hb, wqkv_ref[...], preferred_element_type=jnp.float32)
            q_scr[rows, :] = (qkv[:, 0:D] * (DH ** -0.5 * LOG2E)).astype(jnp.bfloat16)
            k_scr[rows, :] = qkv[:, D:2 * D].astype(jnp.bfloat16)
            vt = qkv[:, 2 * D:3 * D].T.astype(jnp.bfloat16)
            for h in range(H):
                vt_scr[h, 0:16, rows] = vt[h * DH:(h + 1) * DH, :]

    qrows = pl.ds(pl.multiple_of(i * tq, tq), tq)
    lane = lax.broadcasted_iota(jnp.int32, (tq, 128), 1) // DH

    def group_body(g, carry):
        gl = pl.ds(pl.multiple_of(g * 128, 128), 128)
        qg = q_scr[qrows, gl]
        kg = k_scr[:, gl]
        for j in range(HG):
            h = g * HG + j
            qm = jnp.where(lane == j, qg, jnp.zeros_like(qg))
            st = lax.dot_general(kg, qm, (((1,), (1,)), ((), ())),
                                 preferred_element_type=jnp.float32)
            m = jnp.max(st, axis=0, keepdims=True)
            pt = jnp.exp2(st - m).astype(jnp.bfloat16)
            r = jnp.dot(vt_scr[h], pt, preferred_element_type=jnp.float32)
            ot_scr[pl.ds(pl.multiple_of(h * DH, DH), DH), :] = r[0:DH, :] / r[DH:DH + 1, :]
        return carry

    lax.fori_loop(0, NG, group_body, 0)

    ga = mod_scr[0:1, 2 * D:3 * D]
    sb = mod_scr[0:1, 3 * D:4 * D]
    cb = mod_scr[0:1, 4 * D:5 * D]
    gb = mod_scr[0:1, 5 * D:6 * D]
    o = ot_scr[...].T.astype(jnp.bfloat16)
    y = jnp.dot(o, wo_ref[...], preferred_element_type=jnp.float32)
    x1 = x_ref[qrows, :].astype(jnp.float32) + ga * y
    h2 = (_ln(x1) * (1.0 + cb) + sb).astype(jnp.bfloat16)
    u = jnp.dot(h2, w1_ref[...], preferred_element_type=jnp.float32) + b1_ref[...].astype(jnp.float32)
    u = jnp.maximum(u, 0.0)
    u = (u * u).astype(jnp.bfloat16)
    z = jnp.dot(u, w2_ref[...], preferred_element_type=jnp.float32) + b2_ref[...].astype(jnp.float32)
    o_ref[...] = (x1 + gb * z).astype(o_ref.dtype)


@jax.jit
def pallas_adaLN_cond__mha_block__dense_activation_squared_relu__prompt_kernel(
        A_x, A_wqkv, A_wo, B_x, B_w1, B_b1, B_w2, B_b2, c, w_mod):
    tq, tp = 512, 512
    x = A_x.reshape(S, D)
    c8 = jnp.broadcast_to(c, (8, D))
    full = lambda shape: pl.BlockSpec(shape, lambda i: (0,) * len(shape))
    out = pl.pallas_call(
        functools.partial(_kernel, tq=tq, tp=tp),
        grid=(S // tq,),
        in_specs=[full((S, D)), full((D, 3 * D)), full((D, D)), full((D, F)), full((1, F)),
                  full((F, D)), full((1, D)), full((8, D)), full((D, 6 * D))],
        out_specs=pl.BlockSpec((tq, D), lambda i: (i, 0)),
        out_shape=jax.ShapeDtypeStruct((S, D), A_x.dtype),
        scratch_shapes=[
            pltpu.VMEM((8, 6 * D), jnp.float32),
            pltpu.VMEM((S, D), jnp.bfloat16),
            pltpu.VMEM((S, D), jnp.bfloat16),
            pltpu.VMEM((H, 32, S), jnp.bfloat16),
            pltpu.VMEM((D, tq), jnp.float32),
        ],
        compiler_params=pltpu.CompilerParams(
            dimension_semantics=("arbitrary",), vmem_limit_bytes=100 * 1024 * 1024),
    )(x, A_wqkv, A_wo, B_w1, B_b1.reshape(1, F), B_w2, B_b2.reshape(1, D), c8, w_mod)
    return out.reshape(1, S, D)
```

```python
import functools
import math

import jax
import jax.numpy as jnp
from jax import lax
import jax.experimental.pallas as pl
import jax.experimental.pallas.tpu as pltpu

S = 2048
D = 512
H = 32
DH = 16
F = 1792
HG = 128 // DH
NG = H // HG
EPS = 1e-5
LOG2E = math.log2(math.e)


def _ln(x):
    m = jnp.mean(x, axis=-1, keepdims=True)
    xc = x - m
    v = jnp.mean(xc * xc, axis=-1, keepdims=True)
    return xc * lax.rsqrt(v + EPS)


def _kernel(x_hbm, wqkv_hbm, wo_hbm, w1_hbm, b1_ref, w2_hbm, b2_ref, c_ref, wmod_hbm,
            o_ref,
            x_ref, wqkv_ref, wo_ref, w1_ref, w2_ref, wmod_ref, sems,
            mod_scr, qt_scr, k_scr, vt_scr, ot_scr, sta_scr, stb_scr, m_scr, mxp_scr,
            *, tq, tp, kc, hu, lag, dep):
    i = pl.program_id(0)
    nq = pl.num_programs(0)
    nc = S // kc
    npc = S // tp
    sub = lax.broadcasted_iota(jnp.int32, (128, tq), 0) // DH

    cp_mod0 = pltpu.make_async_copy(wmod_hbm.at[:, 0:2 * D], wmod_ref.at[:, 0:2 * D], sems.at[0])
    cp_mod1 = pltpu.make_async_copy(wmod_hbm.at[:, 2 * D:6 * D], wmod_ref.at[:, 2 * D:6 * D], sems.at[1])
    cp_wo = pltpu.make_async_copy(wo_hbm, wo_ref, sems.at[2])
    cp_w1 = pltpu.make_async_copy(w1_hbm, w1_ref, sems.at[3])
    cp_w2 = pltpu.make_async_copy(w2_hbm, w2_ref, sems.at[4])
    cp_wqkv = [pltpu.make_async_copy(wqkv_hbm.at[:, pl.ds(t * D, D)], wqkv_ref.at[:, pl.ds(t * D, D)],
                                     sems.at[5 + t]) for t in range(3)]
    cp_x = [pltpu.make_async_copy(x_hbm.at[pl.ds(r * tp, tp), :], x_ref.at[pl.ds(r * tp, tp), :],
                                  sems.at[8 + r]) for r in range(npc)]

    def make_qm(hh):
        h = hh % H
        blk = jnp.minimum(i + hh // H, nq - 1)
        g = h // HG
        j = h % HG
        qg = qt_scr[pl.ds(pl.multiple_of(g * 128, 128), 128), pl.ds(pl.multiple_of(blk * tq, tq), tq)]
        return jnp.where(sub == j, qg, jnp.zeros_like(qg))

    def stage_a(hh, qm, dst, c, mx):
        rows = pl.ds(c * kc, kc)
        st = jnp.dot(k_scr[(hh % H) // HG, rows, :], qm, preferred_element_type=jnp.float32)
        dst[rows, :] = st
        return jnp.maximum(mx, jnp.max(st.reshape(kc // 8, 8, tq), axis=0))

    neg = lambda: jnp.full((8, tq), -jnp.inf, jnp.float32)

    def silu_c():
        c = jnp.broadcast_to(c_ref[...].astype(jnp.float32), (8, D))
        return (c * jax.nn.sigmoid(c)).astype(jnp.bfloat16)

    @pl.when(i == 0)
    def _prologue():
        cp_mod0.start()
        cp_x[0].start()
        for t in range(3):
            cp_wqkv[t].start()

        sc = silu_c()
        cp_mod0.wait()
        mod = jnp.dot(sc, wmod_ref[:, 0:2 * D], preferred_element_type=jnp.float32)
        mod_scr[:, 0:2 * D] = mod.astype(jnp.bfloat16).astype(jnp.float32)
        sa = mod_scr[0:1, 0 * D:1 * D]
        ca = mod_scr[0:1, 1 * D:2 * D]
        for r in range(npc):
            rows = pl.ds(r * tp, tp)
            cp_x[r].wait()
            xb = x_ref[rows, :].astype(jnp.float32)
            hb = (_ln(xb) * (1.0 + ca) + sa).astype(jnp.bfloat16)
            if r == npc - 1:
                cp_mod1.start()
                cp_wo.start()
                cp_w1.start()
                cp_w2.start()
            if r == 0:
                cp_wqkv[0].wait()
            q = jnp.dot(hb, wqkv_ref[:, 0:D], preferred_element_type=jnp.float32)
            qt_scr[:, rows] = (q * (DH ** -0.5 * LOG2E)).T.astype(jnp.bfloat16)
            if r == 0:
                cp_wqkv[1].wait()
            k = jnp.dot(hb, wqkv_ref[:, D:2 * D], preferred_element_type=jnp.float32)
            for g in range(NG):
                k_scr[g, rows, :] = k[:, g * 128:(g + 1) * 128].astype(jnp.bfloat16)
            if r == 0:
                cp_wqkv[2].wait()
                for rr in range(1, npc):
                    cp_x[rr].start()
            v = jnp.dot(hb, wqkv_ref[:, 2 * D:3 * D], preferred_element_type=jnp.float32)
            vt_scr[:, rows] = v.T.astype(jnp.bfloat16)
        qm = make_qm(0)
        mx = neg()
        for c in range(nc):
            mx = stage_a(0, qm, sta_scr, c, mx)
        m_scr[...] = jnp.max(mx, axis=0, keepdims=True)
        qm = make_qm(1)
        mx = neg()
        for c in range(lag):
            mx = stage_a(1, qm, stb_scr, c, mx)
        mxp_scr[...] = mx

    def one_head(h, cur, nxt, mx1, m, prev):
        qm1 = make_qm(h + 1)
        qm2 = make_qm(h + 2)
        hrows = pl.ds(pl.multiple_of(h * DH, DH), DH)
        mx2 = neg()
        acc = jnp.zeros((DH, tq), jnp.float32)
        l = jnp.zeros((8, tq), jnp.float32)
        m_next = None
        accs = list(prev[-dep:]) if prev else []
        off = len(accs)
        for c in range(nc):
            ca = c + lag
            if ca < nc:
                mx1 = stage_a(h + 1, qm1, nxt, ca, mx1)
                if ca == nc - 1:
                    m_next = jnp.max(mx1, axis=0, keepdims=True)
            else:
                mx2 = stage_a(h + 2, qm2, cur, ca - nc, mx2)
            rows = pl.ds(c * kc, kc)
            mc = m if c + off < dep else m + accs[c + off - dep][0:1, :] * 0.0
            p = jnp.exp2(cur[rows, :] - mc)
            l = l + jnp.sum(p.reshape(kc // 8, 8, tq), axis=0)
            acc = acc + jnp.dot(vt_scr[hrows, rows], p.astype(jnp.bfloat16),
                                preferred_element_type=jnp.float32)
            accs.append(acc)
        ot_scr[hrows, :] = acc / jnp.sum(l, axis=0, keepdims=True)
        return mx2, m_next, accs

    def head_body(p, carry):
        mx = mxp_scr[...]
        m = m_scr[...]
        prev = []
        for u in range(hu // 2):
            mx, m, prev = one_head(hu * p + 2 * u, sta_scr, stb_scr, mx, m, prev)
            mx, m, prev = one_head(hu * p + 2 * u + 1, stb_scr, sta_scr, mx, m, prev)
        mxp_scr[...] = mx
        m_scr[...] = m
        return carry

    lax.fori_loop(0, H // hu, head_body, 0)

    @pl.when(i == 0)
    def _wait_weights():
        cp_mod1.wait()
        mod = jnp.dot(silu_c(), wmod_ref[:, 2 * D:6 * D], preferred_element_type=jnp.float32)
        mod_scr[:, 2 * D:6 * D] = mod.astype(jnp.bfloat16).astype(jnp.float32)
        cp_wo.wait()
        cp_w1.wait()
        cp_w2.wait()

    qrows = pl.ds(pl.multiple_of(i * tq, tq), tq)
    ga = mod_scr[0:1, 2 * D:3 * D]
    sb = mod_scr[0:1, 3 * D:4 * D]
    cb = mod_scr[0:1, 4 * D:5 * D]
    gb = mod_scr[0:1, 5 * D:6 * D]
    o = ot_scr[...].T.astype(jnp.bfloat16)
    y = jnp.dot(o, wo_ref[...], preferred_element_type=jnp.float32)
    x1 = x_ref[qrows, :].astype(jnp.float32) + ga * y
    h2 = (_ln(x1) * (1.0 + cb) + sb).astype(jnp.bfloat16)
    u = jnp.dot(h2, w1_ref[...], preferred_element_type=jnp.float32) + b1_ref[...].astype(jnp.float32)[None, :]
    u = jnp.maximum(u, 0.0)
    u = (u * u).astype(jnp.bfloat16)
    z = jnp.dot(u, w2_ref[...], preferred_element_type=jnp.float32) + b2_ref[...].astype(jnp.float32)[None, :]
    o_ref[...] = (x1 + gb * z).astype(o_ref.dtype)


@jax.jit
def pallas_adaLN_cond__mha_block__dense_activation_squared_relu__prompt_kernel(
        A_x, A_wqkv, A_wo, B_x, B_w1, B_b1, B_w2, B_b2, c, w_mod):
    tq = 256
    tp = 512
    kc = 128
    hu = 16
    lag = 4
    dep = 6
    x = A_x.reshape(S, D)
    full = lambda shape: pl.BlockSpec(shape, lambda i: (0,) * len(shape))
    hbm = pl.BlockSpec(memory_space=pl.ANY)
    bf = jnp.bfloat16
    out = pl.pallas_call(
        functools.partial(_kernel, tq=tq, tp=tp, kc=kc, hu=hu, lag=lag, dep=dep),
        grid=(S // tq,),
        in_specs=[hbm, hbm, hbm, hbm, full((F,)), hbm, full((D,)), full((1, D)), hbm],
        out_specs=pl.BlockSpec((tq, D), lambda i: (i, 0)),
        out_shape=jax.ShapeDtypeStruct((S, D), A_x.dtype),
        scratch_shapes=[
            pltpu.VMEM((S, D), bf),
            pltpu.VMEM((D, 3 * D), bf),
            pltpu.VMEM((D, D), bf),
            pltpu.VMEM((D, F), bf),
            pltpu.VMEM((F, D), bf),
            pltpu.VMEM((D, 6 * D), bf),
            pltpu.SemaphoreType.DMA((8 + S // tp,)),
            pltpu.VMEM((8, 6 * D), jnp.float32),
            pltpu.VMEM((D, S), bf),
            pltpu.VMEM((NG, S, 128), bf),
            pltpu.VMEM((D, S), bf),
            pltpu.VMEM((D, tq), jnp.float32),
            pltpu.VMEM((S, tq), jnp.float32),
            pltpu.VMEM((S, tq), jnp.float32),
            pltpu.VMEM((1, tq), jnp.float32),
            pltpu.VMEM((8, tq), jnp.float32),
        ],
        compiler_params=pltpu.CompilerParams(
            dimension_semantics=("arbitrary",), vmem_limit_bytes=100 * 1024 * 1024),
    )(x, A_wqkv, A_wo, B_w1, B_b1, B_w2, B_b2, c, w_mod)
    return out.reshape(1, S, D)
```
